```python
import os as _os
_os.environ.setdefault("JAX_PLATFORMS", "cpu")
import jax
import jax.numpy as jnp

def _softmax(x, axis=-1):
    return jax.nn.softmax(x, axis=axis)
def _gelu(x):
    return jax.nn.gelu(x, approximate=True)
def _silu(x):
    return jax.nn.silu(x)
def _sigmoid(x):
    return jax.nn.sigmoid(x)
def _layernorm(x, axis=-1, eps=1e-5):
    m = jnp.mean(x, axis=axis, keepdims=True)
    v = jnp.var(x, axis=axis, keepdims=True)
    return (x - m) / jnp.sqrt(v + eps)
def _scatter_add(tgt, idx, src, axis=0):
    return tgt.at[idx].add(src)
def _segment_sum(src, seg, n):
    return jax.ops.segment_sum(src, seg, n)
class _Rng:
    def __init__(self, key):
        self._k = key
    def _next(self):
        self._k, sub = jax.random.split(self._k)
        return sub
    def normal(self, shape):
        return jax.random.normal(self._next(), shape, dtype=jnp.bfloat16)
    def randint(self, lo, hi, shape):
        return jax.random.randint(self._next(), shape, lo, hi, dtype=jnp.int32)
    def uniform(self, shape, lo=0.0, hi=1.0):
        return jax.random.uniform(self._next(), shape, jnp.bfloat16, lo, hi)
    def permutation(self, n):
        return jax.random.permutation(self._next(), n)


kernel_name = 'gated_mix__sliding_block__sliding_local_dilated__prompt'

def setup_inputs():
    _rng = _Rng(jax.random.key(int.from_bytes(__import__("os").urandom(4), "little")))
    _w = (lambda a: (lambda t: t.astype(jnp.bfloat16) if jnp.issubdtype(t.dtype, jnp.floating) else t)(jnp.asarray(a)))
    def _A_setup():
        B, S, D = 1, 2048, 640
        return {
            "x": _w((lambda *s: _rng.normal(s) * 0.05)(B, S, D)),
            "wqkv": _w((lambda *s: _rng.normal(s) * 0.8)(D, 3 * D)),
            "wo": _w((lambda *s: _rng.normal(s) * 0.05)(D, D)),
        }
    _A_in = _A_setup()

    def _B_setup():
        B, S, D = 1, 2048, 640
        return {
            "x": _w((lambda *s: _rng.normal(s) * 0.05)(B, S, D)),
            "wqkv": _w((lambda *s: _rng.normal(s) * 0.8)(D, 3 * D)),
            "wo": _w((lambda *s: _rng.normal(s) * 0.05)(D, D)),
        }
    _B_in = _B_setup()

    return {
        "A_x": _A_in["x"],
        "A_wqkv": _A_in["wqkv"],
        "A_wo": _A_in["wo"],
        "B_x": _B_in["x"],
        "B_wqkv": _B_in["wqkv"],
        "B_wo": _B_in["wo"],
        "gate_w": _w((lambda *s: _rng.normal(s) * 0.05)(640) * 16.0),
    }

def reference(A_x, A_wqkv, A_wo, B_x, B_wqkv, B_wo, gate_w):
    def _A_ref(x, wqkv, wo):
        B, S, D = x.shape
        H = 32; Dh = D // H; W = 256
        qkv = (lambda x, *d: x.transpose(*d))((x @ wqkv).reshape(B, S, 3, H, Dh), 2, 0, 3, 1, 4)
        q, k, v = qkv[0], qkv[1], qkv[2]
        scores = jnp.einsum("bhqd,bhkd->bhqk", q, k) * (Dh ** -0.5)
        idx = jnp.arange(S)
        mask = (idx[:, None] - idx[None, :] >= 0) & (idx[:, None] - idx[None, :] < W)
        scores = jnp.where(mask[None, None], scores, -1e9)
        p = _softmax(scores, axis=-1)
        o = jnp.einsum("bhqk,bhkd->bhqd", p, v)
        return (lambda x, *d: x.transpose(*d))(o, 0, 2, 1, 3).reshape(B, S, D) @ wo

    def _B_ref(x, wqkv, wo):
        B, S, D = x.shape
        H = 32; Dh = D // H
        W, dil = 8, 2
        qkv = (lambda x, *d: x.transpose(*d))((x @ wqkv).reshape(B, S, 3, H, Dh), 2, 0, 3, 1, 4)
        q, k, v = qkv[0], qkv[1], qkv[2]
        scale = Dh ** -0.5
        pos = jnp.arange(S)
        off = jnp.arange(W) * dil
        idx = pos[:, None] - off[None, :]
        mask = idx >= 0
        idx_c = jnp.where(mask, idx, 0).reshape(-1)
        kg = k[:, :, idx_c, :].reshape(B, H, S, W, Dh)
        vg = v[:, :, idx_c, :].reshape(B, H, S, W, Dh)
        logits = jnp.einsum("bhsd,bhswd->bhsw", q, kg) * scale
        logits = jnp.where(mask[None, None, :, :], logits, -1e9)
        attn = _softmax(logits, axis=-1)
        o = jnp.einsum("bhsw,bhswd->bhsd", attn, vg)
        return (lambda x, *d: x.transpose(*d))(o, 0, 2, 1, 3).reshape(B, S, D) @ wo

    x = A_x
    g = _sigmoid((x * gate_w).sum(-1, keepdims=True))
    a = _A_ref(x, A_wqkv, A_wo)
    b = _B_ref(x, B_wqkv, B_wo)
    return g * a + (1 - g) * b
```

```python
import functools
import jax
import jax.numpy as jnp
import numpy as np
from jax import lax
import jax.experimental.pallas as pl
import jax.experimental.pallas.tpu as pltpu

S = 2048
D = 640
H = 32
DH = 20
WA = 256
BM = 512
QT = 128
NEG = -1e30
LOG2E = 1.4426950408889634
SCALE = float(DH ** -0.5)
L_LO, L_HI = 2.0 ** -30, 2.0 ** 64
HB = 16

NN = (((1,), (0,)), ((), ()))
NT = (((1,), (1,)), ((), ()))
f32 = jnp.float32
bf16 = jnp.bfloat16
u32 = jnp.uint32


def _dot(a, b, dn=NN):
    return lax.dot_general(a, b, dn, preferred_element_type=f32)


def _batches():
    out, cur, n = [], [], 0
    for h in range(H):
        lo, hi = h * DH, h * DH + DH
        j0, j1 = lo // 128, (hi - 1) // 128
        cur.append((h, j0 * 128, (j1 + 1) * 128))
        n += j1 - j0 + 1
        if n == 4:
            out.append(cur)
            cur, n = [], 0
    assert not cur
    return out


def _interleave(*streams):
    streams = [list(s) for s in streams if s]
    if not streams:
        return
    n = max(len(s) for s in streams)
    pos = [0] * len(streams)
    for i in range(n):
        for k, s in enumerate(streams):
            tgt = ((i + 1) * len(s) + n - 1) // n
            while pos[k] < tgt:
                s[pos[k]]()
                pos[k] += 1


def kernel(xa_ref, wa_h, woa_h, wb_h, wob_h, gw_ref, o_ref,
           wa_ref, woa_ref, wb_ref, wob_ref, sem,
           wvt_s, wbt_s, wobp_s, tmp_s, ka_s, vt_s, kb_s, vb_s, bias_s, ot_s, qm_s, s_s, q_s, p_s, qb_s, ob_s, oa_s):
    i = pl.program_id(0)

    cps = [pltpu.make_async_copy(h_, v_, sem.at[n]) for n, (h_, v_) in
           enumerate(((wa_h, wa_ref), (wb_h, wb_ref), (wob_h, wob_ref), (woa_h, woa_ref)))]

    @pl.when(i == 0)
    def _init():
        for cp in cps:
            cp.start()
        row = lax.broadcasted_iota(jnp.int32, (QT, QT), 0)
        col = lax.broadcasted_iota(jnp.int32, (QT, QT), 1)
        bias_s[2] = jnp.where(row <= col, 0.0, NEG)
        bias_s[3] = jnp.where(row > col, 0.0, NEG)
        ka_s[:, 0:WA // 2, :] = jnp.zeros((8, WA // 2, 128), u32)
        vt_s[0:2] = jnp.zeros((2, D, 128), bf16)
        kb_s[:, 0:HB, :] = jnp.zeros((5, HB, 128), f32)
        vb_s[:, 0:HB, :] = jnp.zeros((5, HB, 128), f32)
        cps[0].wait()
        wvt_s[...] = wa_ref[:, 2 * D:3 * D].astype(f32).T.astype(bf16)

    r0 = pl.multiple_of(i * BM, BM)
    z = lax.div(i, 64)
    lane = lax.broadcasted_iota(jnp.int32, (1, 128), 1)

    def pad4(get, g):
        j0, o = divmod(80 * g, 128)
        t0 = get(j0)
        if o == 0:
            return t0
        if o + 80 > 128:
            t0 = jnp.where(lane >= o, t0, get(j0 + 1))
        return pltpu.roll(t0, 128 - o, 1)

    RU = 128
    cache = {}
    def getter(c, u):
        def get(j):
            if (c, j, u) not in cache:
                y = _dot(xa_ref[u * RU:(u + 1) * RU, :], wa_ref[:, c * D + j * 128:c * D + (j + 1) * 128])
                cache[c, j, u] = y * (SCALE * LOG2E) if c == 0 else y
            return cache[c, j, u]
        return get
    for u in range(BM // RU):
        for g in range(8):
            qp = pad4(getter(0, u), g)
            for hi in range(4):
                msk = (lane >= hi * DH) & (lane < hi * DH + DH)
                qm_s[z + u * 8 + g, hi * 128:(hi + 1) * 128, :] = jnp.where(msk, qp, 0.0).astype(bf16)
        for g in range(8):
            ka_s[g, pl.ds(pl.multiple_of((r0 + WA + u * RU) // 2, RU // 2), RU // 2), :] = pltpu.bitcast(pad4(getter(1, u), g).astype(bf16), u32)
    for j in range(5):
        vta = _dot(wvt_s[j * 128:(j + 1) * 128, :], xa_ref[...], NT).astype(bf16)
        for c in range(BM // 128):
            vt_s[(BM // QT) * i + 2 + c, j * 128:(j + 1) * 128, :] = vta[:, c * 128:(c + 1) * 128]

    sub = lax.broadcasted_iota(jnp.int32, (8, 128), 0)
    NB = 8
    state = {}

    def p1_steps(t, b):
        q0 = r0 + t * QT
        par = (t * NB + b) % 2
        steps = []

        def prep():
            if b == 0:
                pen0 = jnp.where(q0 >= 256, 0.0, NEG)
                pen1 = jnp.where(q0 >= 128, 0.0, NEG)
                bias_s[0 + 4 * t] = jnp.minimum(bias_s[3], pen0)
                bias_s[1 + 4 * t] = jnp.zeros((QT, QT), f32) + pen1
        steps.append(prep)
        for rc in range(3):
            def step(rc=rc):
                kk = pltpu.bitcast(ka_s[b, pl.ds(pl.multiple_of((q0 + rc * 128) // 2, 64), 64), :], bf16)
                sall = _dot(kk, qm_s[z + t * 8 + b], NT)
                for hi in range(4):
                    h = 4 * b + hi
                    s = sall[:, hi * 128:(hi + 1) * 128]
                    s = s + (bias_s[2] if rc == 2 else bias_s[rc + 4 * t])
                    p = jnp.exp2(s)
                    l = jnp.sum(p.reshape(16, 8, 128), axis=0)
                    p_s[par, hi, rc * 128:(rc + 1) * 128, :] = p.astype(bf16)
                    state['l', t, h] = l if rc == 0 else state['l', t, h] + l
            steps.append(step)
        return steps

    def p2_steps(t, b):
        par = (t * NB + b) % 2
        steps = []
        for hi in range(4):
            h = 4 * b + hi
            w0 = 80 * b + 16 * hi
            for rc in range(3):
                def step(rc=rc, hi=hi, h=h):
                    if rc == 0:
                        m = state.pop(('m', t, h))
                        m = jnp.max(m, axis=0, keepdims=True)
                        state['mb', t, h] = jnp.broadcast_to(m, (8, 128))
                    m = state['mb', t, h]
                    s = s_s[par, hi, rc * 128:(rc + 1) * 128, :].reshape(16, 8, 128)
                    p = jnp.exp2(s - m[None])
                    l = jnp.sum(p, axis=0)
                    p_s[par, hi, rc * 128:(rc + 1) * 128, :] = p.reshape(128, 128).astype(bf16)
                    state['l', t, h] = l if rc == 0 else state['l', t, h] + l

                def stepb(rc=rc, hi=hi, h=h, w0=w0):
                    vt = vt_s[(BM // QT) * i + t + rc, w0:w0 + 32, :]
                    o = _dot(vt, p_s[par, hi, rc * 128:(rc + 1) * 128, :])
                    state['o', t, h] = o if rc == 0 else state['o', t, h] + o
                    if rc == 2:
                        l = jnp.sum(state.pop(('l', t, h)), axis=0, keepdims=True)
                        o = state.pop(('o', t, h))
                        ok = jnp.where((l >= L_LO) & (l <= L_HI), 1.0, 0.0)
                        state['ok'] = ok if 'ok' not in state else jnp.minimum(state['ok'], ok)
                        a = (20 * hi - 16 * hi) // 8
                        o = o[8 * a:8 * a + 24] * (1.0 / l)
                        base = 40 * (h // 2)
                        if h % 2 == 0:
                            ot_s[t, base:base + 16, :] = o[0:16]
                            state['carry', t] = o[16:24]
                        else:
                            ot_s[t, base + 16:base + 24, :] = jnp.where(sub < 4, state.pop(('carry', t)), o[0:8])
                            ot_s[t, base + 24:base + 40, :] = o[8:24]
                steps.append((step, stepb))
        return steps

    NT_ = BM // QT
    NK = NT_ * NB
    def bproj(c, j):
        def f():
            y = _dot(xa_ref[...], wbt_s[c * D + j * 128:c * D + (j + 1) * 128, :], NT)
            if c == 0:
                qb_s[j] = y * (SCALE * LOG2E)
            elif c == 1:
                kb_s[j, pl.ds(r0 + HB, BM), :] = y
            else:
                vb_s[j, pl.ds(r0 + HB, BM), :] = y
        return f

    RB = 32
    def battn(r):
        def f():
            rr = r0 + r * RB
            pos = lax.broadcasted_iota(jnp.int32, (RB, 128), 0) + rr
            lg = []
            qb = [qb_s[j, r * RB:(r + 1) * RB, :] for j in range(5)]
            for w in range(8):
                acc = None
                for j in range(5):
                    pr = qb[j] * kb_s[j, pl.ds(rr + HB - 2 * w, RB), :]
                    acc = pr if acc is None else acc + pr
                acc = acc + pltpu.roll(acc, 64, 1)
                acc = acc + pltpu.roll(acc, 32, 1)
                if w > 0 and r * RB < 2 * w:
                    acc = jnp.where(pos >= 2 * w, acc, NEG)
                lg.append(acc)
            m = functools.reduce(jnp.maximum, lg)
            ps = [jnp.exp2(x - m) for x in lg]
            inv = 1.0 / functools.reduce(lambda x, y: x + y, ps)
            for j in range(5):
                acc = None
                for w in range(8):
                    pr = ps[w] * vb_s[j, pl.ds(rr + HB - 2 * w, RB), :]
                    acc = pr if acc is None else acc + pr
                ob_s[r * RB:(r + 1) * RB, j * 128:(j + 1) * 128] = (acc * inv).astype(bf16)
        return f

    def gate(t):
        xt = xa_ref[t * QT:(t + 1) * QT, :].astype(f32)
        return jax.nn.sigmoid(jnp.sum(xt * gw_ref[...].astype(f32), axis=1, keepdims=True))

    def oa_prep(t):
        def f():
            oa_s[t] = ot_s[t].T.astype(bf16)
            state['g', t] = gate(t)
        return f

    def oproj(t, j):
        def f():
            cs = slice(j * 128, (j + 1) * 128)
            a = _dot(oa_s[t], woa_ref[:, cs])
            b = _dot(ob_s[t * QT:(t + 1) * QT, :], wobp_s[:, cs])
            g = state['g', t]
            o_ref[t * QT:(t + 1) * QT, cs] = (g * a + (1.0 - g) * b).astype(o_ref.dtype)
        return f

    @pl.when(i == 0)
    def _initb():
        cps[1].wait()
        for c in range(3):
            t = wb_ref[:, c * D:(c + 1) * D].astype(f32).T
            for j in range(5):
                tmp_s[j] = t[:, j * 128:(j + 1) * 128]
            for j in range(5):
                for d in range(DH):
                    blk = tmp_s[j, pl.ds(d, H, stride=DH), :]
                    wbt_s[pl.ds(c * D + d * H, H), j * 128:(j + 1) * 128] = blk.astype(bf16)

    for c in (1, 0, 2):
        for j in range(5):
            bproj(c, j)()
    fill = {k: [] for k in range(NK + 2)}
    for r in range(BM // RB):
        fill[1 + 2 * r].append(battn(r))
    for k in range(NK + 1):
        s1 = p1_steps(k // NB, k % NB) if k < NK else []
        s3 = [b_ for _, b_ in p2_steps((k - 1) // NB, (k - 1) % NB)] if k > 0 else []
        if s1:
            s1[0]()
            s1 = s1[1:]
        for n in range(12):
            if n % 4 == 0 and n // 4 < len(s1):
                s1[n // 4]()
            if n < len(s3):
                s3[n]()
            if n == 5:
                for f in fill[k]:
                    f()
    @pl.when(jnp.min(state['ok']) < 0.5)
    def _true_max():
        def body(n, _):
            t, b = n // NB, n % NB
            q0 = pl.multiple_of(r0 + t * QT, QT)
            sall = []
            for rc in range(3):
                kk = pltpu.bitcast(ka_s[b, pl.ds(pl.multiple_of((q0 + rc * 128) // 2, 64), 64), :], bf16)
                bias = bias_s[2] if rc == 2 else bias_s[rc + 4 * t]
                sall.append(_dot(kk, qm_s[n], NT) + jnp.concatenate([bias] * 4, axis=1))
            m = jnp.max(jnp.maximum(jnp.maximum(sall[0], sall[1]), sall[2]), axis=0, keepdims=True)
            ps = [jnp.exp2(x - m) for x in sall]
            l = jnp.sum(ps[0] + ps[1] + ps[2], axis=0, keepdims=True)
            os_ = []
            for hi in range(4):
                cs = slice(hi * 128, (hi + 1) * 128)
                o = sum(_dot(vt_s[(BM // QT) * i + t + rc, pl.ds(pl.multiple_of(80 * b + 16 * hi, 16), 32), :],
                             ps[rc][:, cs].astype(bf16)) for rc in range(3))
                os_.append(o * (1.0 / l[:, cs]))
            o0, o1, o2, o3 = os_
            ot_s[t, pl.ds(pl.multiple_of(80 * b, 16), 80), :] = jnp.concatenate([
                o0[0:16], jnp.where(sub < 4, o0[16:24], o1[0:8]), o1[8:24],
                o2[8:24], jnp.where(sub < 4, o2[24:32], o3[8:16]), o3[16:32]], axis=0)
            return 0
        lax.fori_loop(0, NK, body, 0)

    @pl.when(i == 0)
    def _inito():
        cps[2].wait()
        cps[3].wait()
        t = wob_ref[...].astype(f32)
        for j in range(5):
            tmp_s[j] = t[:, j * 128:(j + 1) * 128]
        for j in range(5):
            for d in range(DH):
                blk = tmp_s[j, pl.ds(d, H, stride=DH), :]
                wobp_s[pl.ds(d * H, H), j * 128:(j + 1) * 128] = blk.astype(bf16)

    oa_prep(0)()
    for j in range(5):
        oproj(0, j)()
    for t_ in range(1, NT_):
        oa_prep(t_)()
        for j in range(5):
            oproj(t_, j)()


def build(interpret=False):
    def const(shape):
        return pl.BlockSpec(shape, lambda i: (0,) * len(shape), pipeline_mode=pl.Buffered(1))
    return pl.pallas_call(
        kernel,
        grid=(S // BM,),
        in_specs=[
            pl.BlockSpec((BM, D), lambda i: (i, 0)),
            pl.BlockSpec(memory_space=pl.ANY), pl.BlockSpec(memory_space=pl.ANY),
            pl.BlockSpec(memory_space=pl.ANY), pl.BlockSpec(memory_space=pl.ANY), const((1, D)),
        ],
        out_specs=pl.BlockSpec((BM, D), lambda i: (i, 0)),
        out_shape=jax.ShapeDtypeStruct((S, D), bf16),
        scratch_shapes=[
            pltpu.VMEM((D, 3 * D), bf16), pltpu.VMEM((D, D), bf16), pltpu.VMEM((D, 3 * D), bf16), pltpu.VMEM((D, D), bf16),
            pltpu.SemaphoreType.DMA((4,)),
            pltpu.VMEM((D, D), bf16), pltpu.VMEM((3 * D, D), bf16), pltpu.VMEM((D, D), bf16),
            pltpu.VMEM((5, D, 128), f32),
            pltpu.VMEM((8, (WA + S) // 2, 128), u32), pltpu.VMEM(((WA + S) // 128, D, 128), bf16),
            pltpu.VMEM((5, HB + S, 128), f32), pltpu.VMEM((5, HB + S, 128), f32),
            pltpu.VMEM((4 * BM // QT, QT, QT), f32), pltpu.VMEM((BM // QT, D, QT), f32),
            pltpu.VMEM((8 * BM // QT, 4 * QT, 128), bf16), pltpu.VMEM((8, 128), f32),
            pltpu.VMEM((8, BM, 128), f32), pltpu.VMEM((2, 4, 384, QT), bf16),
            pltpu.VMEM((5, BM, 128), f32), pltpu.VMEM((BM, D), bf16), pltpu.VMEM((BM // QT, QT, D), bf16),
        ],
        compiler_params=pltpu.CompilerParams(dimension_semantics=("arbitrary",), vmem_limit_bytes=100 * 1024 * 1024),
        name="gmix",
        interpret=interpret,
    )


def run(A_x, A_wqkv, A_wo, B_x, B_wqkv, B_wo, gate_w, interpret=False):
    out = build(interpret)(A_x.reshape(S, D), A_wqkv, A_wo, B_wqkv, B_wo, gate_w.reshape(1, D))
    return out.reshape(1, S, D)


@jax.jit
def pallas_gated_mix__sliding_block__sliding_local_dilated__prompt_kernel(A_x, A_wqkv, A_wo, B_x, B_wqkv, B_wo, gate_w):
    return run(A_x, A_wqkv, A_wo, B_x, B_wqkv, B_wo, gate_w)
```
